```python
import os as _os
_os.environ.setdefault("JAX_PLATFORMS", "cpu")
import jax
import jax.numpy as jnp

def _softmax(x, axis=-1):
    return jax.nn.softmax(x, axis=axis)
def _gelu(x):
    return jax.nn.gelu(x, approximate=True)
def _silu(x):
    return jax.nn.silu(x)
def _sigmoid(x):
    return jax.nn.sigmoid(x)
def _layernorm(x, axis=-1, eps=1e-5):
    m = jnp.mean(x, axis=axis, keepdims=True)
    v = jnp.var(x, axis=axis, keepdims=True)
    return (x - m) / jnp.sqrt(v + eps)
def _scatter_add(tgt, idx, src, axis=0):
    return tgt.at[idx].add(src)
def _segment_sum(src, seg, n):
    return jax.ops.segment_sum(src, seg, n)
class _Rng:
    def __init__(self, key):
        self._k = key
    def _next(self):
        self._k, sub = jax.random.split(self._k)
        return sub
    def normal(self, shape):
        return jax.random.normal(self._next(), shape, dtype=jnp.bfloat16)
    def randint(self, lo, hi, shape):
        return jax.random.randint(self._next(), shape, lo, hi, dtype=jnp.int32)
    def uniform(self, shape, lo=0.0, hi=1.0):
        return jax.random.uniform(self._next(), shape, jnp.bfloat16, lo, hi)
    def permutation(self, n):
        return jax.random.permutation(self._next(), n)


kernel_name = 'sequential_preLN__softmax_full_mha__mixer_channel_mlp__prompt'

def setup_inputs():
    _rng = _Rng(jax.random.key(int.from_bytes(__import__("os").urandom(4), "little")))
    _w = (lambda a: (lambda t: t.astype(jnp.bfloat16) if jnp.issubdtype(t.dtype, jnp.floating) else t)(jnp.asarray(a)))
    def _A_setup():
        B, S, D = 1, 2048, 1024
        return {
            "x": _w((lambda *s: _rng.normal(s) * 0.05)(B, S, D)),
            "wqkv": _w((lambda *s: _rng.normal(s) * 0.05)(D, 3 * D)),
            "wo": _w((lambda *s: _rng.normal(s) * 0.05)(D, D)),
        }
    _A_in = _A_setup()

    def _B_setup():
        B, S, D, F = 1, 2048, 1024, 3584
        return {
            "x": _w((lambda *s: _rng.normal(s) * 0.05)(B, S, D)),
            "w1": _w((lambda *s: _rng.normal(s) * 0.8)(D, F) * (D ** -0.5)),
            "b1": _w((lambda *s: _rng.normal(s) * 0.8)(F)),
            "w2": _w((lambda *s: _rng.normal(s) * 0.8)(F, D) * (F ** -0.5)),
            "b2": _w((lambda *s: _rng.normal(s) * 0.05)(D)),
        }
    _B_in = _B_setup()

    return {
        "A_x": _A_in["x"],
        "A_wqkv": _A_in["wqkv"],
        "A_wo": _A_in["wo"],
        "B_x": _B_in["x"],
        "B_w1": _B_in["w1"],
        "B_b1": _B_in["b1"],
        "B_w2": _B_in["w2"],
        "B_b2": _B_in["b2"],
    }

def reference(A_x, A_wqkv, A_wo, B_x, B_w1, B_b1, B_w2, B_b2):
    def _A_ref(x, wqkv, wo):
        B, S, D = x.shape
        H = 32; Dh = D // H
        qkv = (lambda x, *d: x.transpose(*d))((x @ wqkv).reshape(B, S, 3, H, Dh), 2, 0, 3, 1, 4)
        q, k, v = qkv[0], qkv[1], qkv[2]
        scale = Dh ** -0.5
        scores = jnp.einsum("bhqd,bhkd->bhqk", q, k) * scale
        p = _softmax(scores, axis=-1)
        o = jnp.einsum("bhqk,bhkd->bhqd", p, v)
        return (lambda x, *d: x.transpose(*d))(o, 0, 2, 1, 3).reshape(B, S, D) @ wo

    def _B_ref(x, w1, b1, w2, b2):
        y = _layernorm(x, axis=-1)
        h = _gelu(jnp.einsum("bsd,df->bsf", y, w1) + b1)
        return jnp.einsum("bsf,fd->bsd", h, w2) + b2

    x = A_x
    h = x + _A_ref(_layernorm(x, axis=-1), A_wqkv, A_wo)
    h2 = h + _B_ref(_layernorm(h, axis=-1), B_w1, B_b1, B_w2, B_b2)
    return h2
```

```python
import functools, math
import contextlib
import jax, jax.numpy as jnp
from jax import lax
from jax.experimental import pallas as pl
from jax.experimental.pallas import tpu as pltpu

S, D, F, H, DH = 2048, 1024, 3584, 32, 32
G = 8
EPS = 1e-5
QSCALE = (DH ** -0.5) * math.log2(math.e)
f32, bf16 = jnp.float32, jnp.bfloat16

def _ln(x):
    m = jnp.mean(x, axis=-1, keepdims=True)
    xc = x - m
    v = jnp.mean(xc * xc, axis=-1, keepdims=True)
    return xc * lax.rsqrt(v + EPS)

def _gelu(x):
    return 0.5 * x * (1.0 + jnp.tanh(0.7978845608028654 * (x + 0.044715 * (x * x * x))))

def _ds(i, n):
    if isinstance(i, int):
        return pl.ds(i * n, n)
    return pl.ds(pl.multiple_of(i * n, n), n)

def make(TM=256, TQ=512, FC=512, KC=128, WC=512, SKEW=0, QKLEAD=False, OPN=128, TM3=256, TOP=256, NEARLY=1,
         scopes=False, PROLOOP=True):
    NT = S // TM
    NQ = S // TQ
    NFC = F // FC
    NIT = NQ * G
    NKC = S // KC
    NWC = 3 * D // WC
    GPC = WC // 128
    NT3 = S // TM3
    NTOP = S // TOP
    scope = (lambda n: jax.named_scope(n)) if scopes else (lambda n: contextlib.nullcontext())

    def kernel(x_hbm, wqkv_hbm, wo_hbm, w1_hbm, b1_ref, w2_hbm, b2_ref, out_hbm,
               x_v, wqkv_v, wo_v, w1_v, w2_v, q_s, k_s, vt_s, o_s, sS, mS, xn_s, y_s, h_s, out_v,
               sem_x, sem_w, sem_r, sem_o):
        rows = lambda t: _ds(t, TM)
        cx = lambda t: pltpu.make_async_copy(x_hbm.at[rows(t), :], x_v.at[rows(t), :], sem_x.at[t])
        cw = [pltpu.make_async_copy(wqkv_hbm.at[:, pl.ds(c * WC, WC)], wqkv_v.at[:, pl.ds(c * WC, WC)], sem_w.at[c]) for c in range(NWC)]
        co = pltpu.make_async_copy(wo_hbm, wo_v, sem_r.at[0])
        c1 = pltpu.make_async_copy(w1_hbm, w1_v, sem_r.at[1])
        c2 = pltpu.make_async_copy(w2_hbm, w2_v, sem_r.at[2])

        def ln_x(t):
            return _ln(x_v[rows(t), :].astype(f32)).astype(bf16)

        def proj(xn, c, t):
            r = jnp.dot(xn, wqkv_v[:, c * WC:(c + 1) * WC], preferred_element_type=f32)
            col0 = c * WC
            if col0 < D:
                for gg in range(GPC):
                    q_s[col0 // 128 + gg, rows(t), :] = (r[:, gg * 128:(gg + 1) * 128] * QSCALE).astype(bf16)
            elif col0 < 2 * D:
                for gg in range(GPC):
                    k_s[(col0 - D) // 128 + gg, rows(t), :] = r[:, gg * 128:(gg + 1) * 128].astype(bf16)
            else:
                vt_s[col0 - 2 * D:col0 - 2 * D + WC, rows(t)] = r.T.astype(bf16)

        with scope('p1_peel'):
            cx(0).start(); cw[0].start(); cw[1].start()
            cx(0).wait()
            xn0 = ln_x(0)
            for c in range(NWC):
                cw[c].wait()
                if c + 2 < NWC:
                    cw[c + 2].start()
                if c == 0:
                    cx(1).start()
                if c == NWC - 3:
                    cx(2).start()
                if c == NWC - 2:
                    for t in range(3, NT):
                        cx(t).start()
                if c == NWC - 1:
                    co.start(); c1.start(); c2.start()
                if c == NWC - 2:
                    cx(1).wait()
                    xn_s[...] = ln_x(1)
                proj(xn0, c, 0)

        def p1(t, carry):
            @pl.when(t + 1 < NT)
            def _():
                cx(t + 1).wait()
            xa = xn_s[...]
            for c in range(NWC):
                proj(xa, c, t)
            xn_s[...] = ln_x(jnp.minimum(t + 1, NT - 1))
            return carry
        with scope('p1_loop'):
            lax.fori_loop(1, NT, p1, 0)

        lane = lax.broadcasted_iota(jnp.int32, (TQ, 128), 1)
        qrows = lambda qi: _ds(qi, TQ)

        def stage(it, do_qk=True, do_pv=True, extra=(), heads=(0, 1, 2, 3)):
            qi = it // G
            g = it % G
            qi_n = (it + 1) // G
            g_n = (it + 1) % G
            st = {}
            outs = []
            P = {}

            def exp_chunk(n):
                jj, c = divmod(n, NKC)
                j = heads[jj]
                if c == 0:
                    st['m'] = mS[j]
                p = jnp.exp2(sS[j, c * KC:(c + 1) * KC, :] - st['m'])
                ls = jnp.sum(p.reshape(KC // 8, 8, TQ), axis=0)
                st['l8', jj] = ls if c == 0 else st['l8', jj] + ls
                P[n] = p.astype(bf16)

            def pv_chunk(n):
                jj, c = divmod(n, NKC)
                j = heads[jj]
                o = jnp.dot(vt_s[_ds(g * 4 + j, DH), c * KC:(c + 1) * KC], P.pop(n), preferred_element_type=f32)
                st['acc'] = o if c == 0 else st['acc'] + o
                if c == NKC - 1:
                    l = jnp.sum(st['l8', jj], axis=0, keepdims=True)
                    outs.append(st['acc'] * (1.0 / l))
                    if j == 3:
                        ot = jnp.concatenate(outs, axis=0)
                        o_s[g, qrows(qi), :] = ot.T.astype(bf16)

            def qk_chunk(n):
                jj, c = divmod(n, NKC)
                j = heads[jj]
                if c == 0:
                    q = q_s[g_n, qrows(qi_n), :]
                    st['qm'] = jnp.where((lane >= j * DH) & (lane < (j + 1) * DH), q, jnp.zeros_like(q))
                s = lax.dot_general(k_s[g_n, c * KC:(c + 1) * KC, :], st['qm'], (((1,), (1,)), ((), ())), preferred_element_type=f32)
                sS[j, c * KC:(c + 1) * KC, :] = s
                ms = jnp.max(s.reshape(KC // 8, 8, TQ), axis=0)
                st['m8'] = ms if c == 0 else jnp.maximum(st['m8'], ms)
                if c == NKC - 1:
                    mS[j] = jnp.max(st['m8'], axis=0, keepdims=True)

            N = len(heads) * NKC
            order = []
            if do_qk and do_pv:
                extra_turns = set(int((k + 1) * N / (SKEW + 1)) for k in range(SKEW))
                iq = ip = ie = 0
                def exp_upto(n):
                    nonlocal ie
                    while ie <= min(n, N - 1):
                        order.append((exp_chunk, ie)); ie += 1
                while iq < N or ip < N:
                    if not QKLEAD and ip < N:
                        exp_upto(ip); order.append((pv_chunk, ip)); ip += 1
                    if iq < N:
                        exp_upto(iq); order.append((qk_chunk, iq)); iq += 1
                    if QKLEAD and ip < N:
                        exp_upto(ip); order.append((pv_chunk, ip)); ip += 1
                        if ip in extra_turns and ip < N:
                            exp_upto(ip); order.append((pv_chunk, ip)); ip += 1
            elif do_qk:
                order = [(qk_chunk, n) for n in range(N)]
            else:
                for n in range(N):
                    order += [(exp_chunk, n), (pv_chunk, n)]
            ne = len(extra)
            ei = 0
            for idx, (f, n) in enumerate(order):
                while ei < ne and ei * len(order) <= idx * ne:
                    extra[ei](); ei += 1
                f(n)
            while ei < ne:
                extra[ei](); ei += 1

        def p2(it, carry):
            stage(it)
            return carry

        def op_piece(t, n, width):
            def f():
                r = _ds(t, TOP)
                o = jnp.concatenate([o_s[g, r, :] for g in range(G)], axis=1)
                cs = slice(n * width, (n + 1) * width)
                h_s[r, cs] = x_v[r, cs].astype(f32) + jnp.dot(o, wo_v[:, cs], preferred_element_type=f32)
            return f

        def ln2(t):
            return _ln(_ln(h_s[_ds(t, TM3), :])).astype(bf16)

        with scope('p2_pro'):
            if PROLOOP:
                def pro(j, carry):
                    stage(-1, do_pv=False, heads=(j,))
                    return carry
                lax.fori_loop(0, 4, pro, 0)
            else:
                stage(-1, do_pv=False)
        with scope('p2_loop'):
            lax.fori_loop(0, NIT - 1, p2, 0)
        with scope('p2_epi'):
            co.wait()
            NOP = D // OPN
            extra = [op_piece(t, n, OPN) for t in range(NEARLY) for n in range(NOP)]
            stage(NIT - 1, do_qk=False, extra=extra)
        with scope('p3a'):
            def p3a(t, carry):
                op_piece(t, 0, D)()
                return carry
            lax.fori_loop(NEARLY, NTOP - 1, p3a, 0)
            y_s[...] = ln2(0)
            op_piece(NTOP - 1, 0, D)()
            c1.wait(); c2.wait()

        def out_copy(t, slot):
            return pltpu.make_async_copy(out_v.at[slot], out_hbm.at[_ds(t, TM3), :], sem_o.at[slot])

        b1 = b1_ref[...].astype(f32).reshape(1, F)
        b2 = b2_ref[...].astype(f32).reshape(1, D)

        def mlp(y, t):
            acc = h_s[_ds(t, TM3), :] + b2
            for c in range(NFC):
                a = jnp.dot(y, w1_v[:, c * FC:(c + 1) * FC], preferred_element_type=f32) + b1[:, c * FC:(c + 1) * FC]
                acc = acc + jnp.dot(_gelu(a).astype(bf16), w2_v[c * FC:(c + 1) * FC, :], preferred_element_type=f32)
            return acc.astype(bf16)

        def p3(t, carry):
            slot = t % 2
            @pl.when(t >= 2)
            def _():
                out_copy(t - 2, slot).wait()
            ya = y_s[...]
            res = mlp(ya, t)
            y_s[...] = ln2(jnp.minimum(t + 1, NT3 - 1))
            out_v[slot] = res
            out_copy(t, slot).start()
            return carry
        with scope('p3b'):
            lax.fori_loop(0, NT3, p3, 0)
            out_copy(NT3 - 2, (NT3 - 2) % 2).wait()
            out_copy(NT3 - 1, (NT3 - 1) % 2).wait()

    @jax.jit
    def fn(A_x, A_wqkv, A_wo, B_x, B_w1, B_b1, B_w2, B_b2):
        x = A_x.reshape(S, D)
        any_spec = pl.BlockSpec(memory_space=pl.ANY)
        vm = pl.BlockSpec(memory_space=pltpu.VMEM)
        out = pl.pallas_call(
            kernel,
            out_shape=jax.ShapeDtypeStruct((S, D), bf16),
            in_specs=[any_spec, any_spec, any_spec, any_spec, vm, any_spec, vm],
            out_specs=any_spec,
            scratch_shapes=[
                pltpu.VMEM((S, D), bf16),
                pltpu.VMEM((D, 3 * D), bf16),
                pltpu.VMEM((D, D), bf16),
                pltpu.VMEM((D, F), bf16),
                pltpu.VMEM((F, D), bf16),
                pltpu.VMEM((G, S, 128), bf16),
                pltpu.VMEM((G, S, 128), bf16),
                pltpu.VMEM((D, S), bf16),
                pltpu.VMEM((G, S, 128), bf16),
                pltpu.VMEM((4, S, TQ), f32),
                pltpu.VMEM((4, 1, TQ), f32),
                pltpu.VMEM((TM, D), bf16),
                pltpu.VMEM((TM3, D), bf16),
                pltpu.VMEM((S, D), f32),
                pltpu.VMEM((2, TM3, D), bf16),
                pltpu.SemaphoreType.DMA((NT,)),
                pltpu.SemaphoreType.DMA((NWC,)),
                pltpu.SemaphoreType.DMA((3,)),
                pltpu.SemaphoreType.DMA((2,)),
            ],
            compiler_params=pltpu.CompilerParams(vmem_limit_bytes=120 * 1024 * 1024),
        )(x, A_wqkv, A_wo, B_w1, B_b1, B_w2, B_b2)
        return out.reshape(1, S, D)
    return fn


_impl = make()


@jax.jit
def pallas_sequential_preLN__softmax_full_mha__mixer_channel_mlp__prompt_kernel(
    A_x: jax.Array,
    A_wqkv: jax.Array,
    A_wo: jax.Array,
    B_x: jax.Array,
    B_w1: jax.Array,
    B_b1: jax.Array,
    B_w2: jax.Array,
    B_b2: jax.Array,
):
    return _impl(A_x, A_wqkv, A_wo, B_x, B_w1, B_b1, B_w2, B_b2)
```

```python
import math

import jax
import jax.numpy as jnp
from jax import lax
from jax.experimental import pallas as pl
from jax.experimental.pallas import tpu as pltpu

S, D, F, H, DH = 2048, 1024, 3584, 32, 32
G = 8
EPS = 1e-5
QSCALE = (DH ** -0.5) * math.log2(math.e)
f32, bf16 = jnp.float32, jnp.bfloat16

TM = 256
WC = 512
NWC = 3 * D // WC
CORDER = (0, 1, 4, 5, 2, 3)
TQ = 512
KC = 128
EPR = 256
OPN = 128
TOP = 256
TM3 = 256
FC = 512
OSPLIT = 4

NT = S // TM
NQ = S // TQ
NIT = NQ * G
NKC = S // KC
NT3 = S // TM3
NFC = F // FC
HN = D // OSPLIT


def _ln(x):
    m = jnp.mean(x, axis=-1, keepdims=True)
    xc = x - m
    v = jnp.mean(xc * xc, axis=-1, keepdims=True)
    return xc * lax.rsqrt(v + EPS)


def _gelu(x):
    return 0.5 * x * (1.0 + jnp.tanh(0.7978845608028654 * (x + 0.044715 * (x * x * x))))


def _ds(i, n):
    if isinstance(i, int):
        return pl.ds(i * n, n)
    return pl.ds(pl.multiple_of(i * n, n), n)


def _dso(start, n, align):
    if isinstance(start, int):
        return pl.ds(start, n)
    return pl.ds(pl.multiple_of(start, align), n)


def _pieces(nrows, n):
    units = nrows // 16
    out, r = [], 0
    for i in range(n):
        u = (units * (i + 1)) // n - (units * i) // n
        if u:
            out.append((r, u * 16))
            r += u * 16
    return out


def _kernel(x_hbm, wqkv_hbm, wo_hbm, w1_hbm, b1_hbm, w2_hbm, b2_hbm, out_hbm,
            x_v, wqkv_v, wo_v, w1_v, w2_v, qvt_s, k_s, o_s, sS, mS, ot_s, xn_s, y_s, h_s, out_v,
            b1_v, b2_v, sem_x, sem_w, sem_r, sem_o):
    rows = lambda t: _ds(t, TM)

    def cx(t):
        return pltpu.make_async_copy(x_hbm.at[rows(t), :], x_v.at[rows(t), :], sem_x.at[t])

    def cw(i):
        if isinstance(i, int):
            c = CORDER[i]
        else:
            c = jnp.where(i < 2, i, jnp.where(i < 4, i + 2, i - 2))
        return pltpu.make_async_copy(wqkv_hbm.at[:, _ds(c, WC)], wqkv_v.at[i], sem_w.at[i])

    co = pltpu.make_async_copy(wo_hbm, wo_v, sem_r.at[0])
    c1 = pltpu.make_async_copy(w1_hbm, w1_v, sem_r.at[1])
    c2 = pltpu.make_async_copy(w2_hbm, w2_v, sem_r.at[2])
    cb1 = pltpu.make_async_copy(b1_hbm, b1_v, sem_r.at[3])
    cb2 = pltpu.make_async_copy(b2_hbm, b2_v, sem_r.at[4])

    def proj(slot, i, t, transposed):
        r = jnp.dot(xn_s[slot], wqkv_v[i], preferred_element_type=f32)
        if transposed:
            if isinstance(i, int):
                if i < 2:
                    r = r * QSCALE
            else:
                r = r * jnp.where(i < 2, QSCALE, 1.0).astype(f32)
            qvt_s[_ds(i, WC), rows(t)] = r.T.astype(bf16)
        else:
            for gg in range(WC // 128):
                k_s[(i - 4) * (WC // 128) + gg, rows(t), :] = r[:, gg * 128:(gg + 1) * 128].astype(bf16)

    def ln_x_piece(t, slot, r0, n):
        xn_s[slot, _dso(r0, n, 16), :] = _ln(x_v[_dso(t * TM + r0, n, 16), :].astype(f32)).astype(bf16)

    cx(0).start()
    cw(0).start()
    cx(0).wait()
    for r0, n in _pieces(TM, 4):
        ln_x_piece(0, 0, r0, n)
    cw(1).start()

    def first_t(i, carry):
        cw(i).wait()
        cw(i + 2).start()

        @pl.when(i == 2)
        def _():
            cx(1).start()
        proj(0, i, 0, True)
        return carry
    lax.fori_loop(0, 4, first_t, 0)
    for t in range(2, NT):
        cx(t).start()
    cx(1).wait()

    def first_k(i, carry):
        cw(i).wait()
        proj(0, i, 0, False)
        ln_x_piece(1, 1, (i - 4) * (TM // 2), TM // 2)
        return carry
    lax.fori_loop(4, 6, first_k, 0)
    co.start()
    c1.start()
    c2.start()
    cb1.start()
    cb2.start()

    def p1(t, carry):
        @pl.when(t + 1 < NT)
        def _():
            cx(t + 1).wait()
        slot = t % 2
        tn = jnp.minimum(t + 1, NT - 1)
        pcs = _pieces(TM, NWC - 1)
        for i in range(NWC):
            proj(slot, i, t, i < 4)
            if i < len(pcs):
                ln_x_piece(tn, 1 - slot, *pcs[i])
        return carry
    lax.fori_loop(1, NT, p1, 0)

    sub = lax.broadcasted_iota(jnp.int32, (128, TQ), 0)
    qrows = lambda qi: _ds(qi, TQ)

    def stage(it, do_qk=True, do_pv=True, extra=(), heads=(0, 1, 2, 3)):
        qi = it // G
        g = it % G
        qi_n = (it + 1) // G
        g_n = (it + 1) % G
        st = {}
        outs = []
        P = {}

        def exp_chunk(n):
            jj, c = divmod(n, NKC)
            j = heads[jj]
            if c == 0:
                st['m'] = jnp.max(mS[j], axis=0, keepdims=True)
            p = jnp.exp2(sS[j, c * KC:(c + 1) * KC, :] - st['m'])
            l8 = None if c == 0 else st['l8', jj]
            for r in reversed(range(KC // 16)):
                pr = p[r * 16:r * 16 + 8, :] + p[r * 16 + 8:r * 16 + 16, :]
                l8 = pr if l8 is None else l8 + pr
            st['l8', jj] = l8
            P[n] = p.astype(bf16)

        def pv_chunk(n):
            jj, c = divmod(n, NKC)
            j = heads[jj]
            o = jnp.dot(qvt_s[_ds(H + g * 4 + j, DH), c * KC:(c + 1) * KC], P.pop(n),
                        preferred_element_type=f32)
            st['acc'] = o if c == 0 else st['acc'] + o
            if c == NKC - 1:
                l = jnp.sum(st['l8', jj], axis=0, keepdims=True)
                res = st['acc'] * (1.0 / l)
                if isinstance(j, int):
                    outs.append(res)
                    if j == 3:
                        ot = jnp.concatenate(outs, axis=0)
                        o_s[g, qrows(qi), :] = ot.T.astype(bf16)
                else:
                    ot_s[_ds(j, DH), :] = res

        def qk_chunk(n):
            jj, c = divmod(n, NKC)
            j = heads[jj]
            if c == 0:
                if isinstance(j, int):
                    qt = qvt_s[_ds(g_n * 4 + j, DH), qrows(qi_n)]
                    parts = []
                    if j > 0:
                        parts.append(jnp.zeros((j * DH, TQ), bf16))
                    parts.append(qt)
                    if j < 3:
                        parts.append(jnp.zeros(((3 - j) * DH, TQ), bf16))
                    st['qm'] = jnp.concatenate(parts, axis=0)
                else:
                    qt = qvt_s[_ds(g_n, 128), qrows(qi_n)]
                    st['qm'] = jnp.where((sub >= j * DH) & (sub < (j + 1) * DH), qt, jnp.zeros_like(qt))
            s = jnp.dot(k_s[g_n, c * KC:(c + 1) * KC, :], st['qm'], preferred_element_type=f32)
            sS[j, c * KC:(c + 1) * KC, :] = s
            ms = jnp.max(s.reshape(KC // 8, 8, TQ), axis=0)
            st['m8'] = ms if c == 0 else jnp.maximum(st['m8'], ms)
            if c == NKC - 1:
                mS[j] = st['m8']

        N = len(heads) * NKC
        order = []
        if do_qk and do_pv:
            ip = 0
            for iq in range(N):
                while ip < N and ip <= iq + (1 if iq >= N // 2 else 0):
                    order += [(exp_chunk, ip), (pv_chunk, ip)]
                    ip += 1
                order.append((qk_chunk, iq))
        elif do_qk:
            order = [(qk_chunk, n) for n in range(N)]
        else:
            for n in range(N):
                order += [(exp_chunk, n), (pv_chunk, n)]
        ne = len(extra)
        ei = 0
        for idx, (fn, n) in enumerate(order):
            while ei < ne and ei * len(order) <= idx * ne:
                extra[ei]()
                ei += 1
            fn(n)
        while ei < ne:
            extra[ei]()
            ei += 1

    def op_piece(r0, nr, c0, nc):
        def fn():
            r = _dso(r0, nr, nr)
            o = jnp.concatenate([o_s[g, r, :] for g in range(G)], axis=1)
            cs = slice(c0, c0 + nc)
            h_s[r, cs] = x_v[r, cs].astype(f32) + jnp.dot(o, wo_v[:, cs], preferred_element_type=f32)
        return fn

    def ln2_piece(t, slot, r0, n):
        y_s[slot, _dso(r0, n, 16), :] = _ln(_ln(h_s[_dso(t * TM3 + r0, n, 16), :])).astype(bf16)

    def prologue(j, carry):
        stage(-1, do_pv=False, heads=(j,))
        return carry
    lax.fori_loop(0, 4, prologue, 0)

    def p2(it, carry):
        stage(it)
        return carry
    lax.fori_loop(0, NIT - 1, p2, 0)

    co.wait()

    def epilogue(j, carry):
        extra = [op_piece(j * EPR, EPR, c0, OPN) for c0 in range(0, D, OPN)]
        stage(NIT - 1, do_qk=False, extra=extra, heads=(j,))
        return carry
    lax.fori_loop(0, 4, epilogue, 0)

    R0 = 4 * EPR
    NOPT = (S - R0) // TOP
    LNR = TM3 // NOPT
    assert R0 + TOP <= S - TQ and TM3 <= R0 and LNR % 16 == 0

    def p3a(i, carry):
        ln2_piece(0, 0, i * LNR, LNR)
        op_piece(R0 + i * TOP, TOP, 0, D)()
        o_s[G - 1, qrows(NQ - 1), :] = ot_s[...].T.astype(bf16)
        return carry
    lax.fori_loop(0, NOPT, p3a, 0)
    c1.wait()
    c2.wait()
    cb1.wait()
    cb2.wait()

    def out_copy(t, slot, hh):
        return pltpu.make_async_copy(out_v.at[slot, :, pl.ds(hh * HN, HN)],
                                     out_hbm.at[_ds(t, TM3), pl.ds(hh * HN, HN)],
                                     sem_o.at[slot * OSPLIT + hh])

    b1 = b1_v[...].astype(f32).reshape(1, F)
    b2 = b2_v[...].astype(f32).reshape(1, D)

    def p3(t, carry):
        slot = t % 2

        @pl.when(t >= 2)
        def _():
            for hh in range(OSPLIT):
                out_copy(t - 2, slot, hh).wait()
        tn = jnp.minimum(t + 1, NT3 - 1)
        pcs = _pieces(TM3, NFC - 1)
        acc = h_s[_ds(t, TM3), :] + b2
        for c in range(NFC):
            fs = slice(c * FC, (c + 1) * FC)
            a = jnp.dot(y_s[slot], w1_v[:, fs], preferred_element_type=f32) + b1[:, fs]
            ga = _gelu(a).astype(bf16)
            if c < NFC - 1:
                acc = acc + jnp.dot(ga, w2_v[fs, :], preferred_element_type=f32)
            else:
                for hh in range(OSPLIT):
                    cs = slice(hh * HN, (hh + 1) * HN)
                    r = acc[:, cs] + jnp.dot(ga, w2_v[fs, cs], preferred_element_type=f32)
                    out_v[slot, :, cs] = r.astype(bf16)
                    out_copy(t, slot, hh).start()
            if c < len(pcs):
                ln2_piece(tn, 1 - slot, *pcs[c])
        return carry
    lax.fori_loop(0, NT3, p3, 0)
    for hh in range(OSPLIT):
        out_copy(NT3 - 2, (NT3 - 2) % 2, hh).wait()
        out_copy(NT3 - 1, (NT3 - 1) % 2, hh).wait()


@jax.jit
def pallas_sequential_preLN__softmax_full_mha__mixer_channel_mlp__prompt_kernel(
    A_x: jax.Array,
    A_wqkv: jax.Array,
    A_wo: jax.Array,
    B_x: jax.Array,
    B_w1: jax.Array,
    B_b1: jax.Array,
    B_w2: jax.Array,
    B_b2: jax.Array,
):
    del B_x
    any_spec = pl.BlockSpec(memory_space=pl.ANY)
    out = pl.pallas_call(
        _kernel,
        out_shape=jax.ShapeDtypeStruct((S, D), bf16),
        in_specs=[any_spec] * 7,
        out_specs=any_spec,
        scratch_shapes=[
            pltpu.VMEM((S, D), bf16),
            pltpu.VMEM((NWC, D, WC), bf16),
            pltpu.VMEM((D, D), bf16),
            pltpu.VMEM((D, F), bf16),
            pltpu.VMEM((F, D), bf16),
            pltpu.VMEM((2 * D, S), bf16),
            pltpu.VMEM((G, S, 128), bf16),
            pltpu.VMEM((G, S, 128), bf16),
            pltpu.VMEM((4, S, TQ), f32),
            pltpu.VMEM((4, 8, TQ), f32),
            pltpu.VMEM((128, TQ), f32),
            pltpu.VMEM((2, TM, D), bf16),
            pltpu.VMEM((2, TM3, D), bf16),
            pltpu.VMEM((S, D), f32),
            pltpu.VMEM((2, TM3, D), bf16),
            pltpu.VMEM((F,), bf16),
            pltpu.VMEM((D,), bf16),
            pltpu.SemaphoreType.DMA((NT,)),
            pltpu.SemaphoreType.DMA((NWC,)),
            pltpu.SemaphoreType.DMA((5,)),
            pltpu.SemaphoreType.DMA((2 * OSPLIT,)),
        ],
        compiler_params=pltpu.CompilerParams(vmem_limit_bytes=100 * 1024 * 1024),
    )(A_x.reshape(S, D), A_wqkv, A_wo, B_w1, B_b1, B_w2, B_b2)
    return out.reshape(1, S, D)
```
